```python
import jax
import jax.numpy as jnp

def _softmax(x, axis=-1):
    return jax.nn.softmax(x, axis=axis)
def _gelu(x):
    return jax.nn.gelu(x, approximate=True)
def _silu(x):
    return jax.nn.silu(x)
def _sigmoid(x):
    return jax.nn.sigmoid(x)
def _layernorm(x, axis=-1, eps=1e-5):
    m = jnp.mean(x, axis=axis, keepdims=True)
    v = jnp.var(x, axis=axis, keepdims=True)
    return (x - m) / jnp.sqrt(v + eps)
def _scatter_add(tgt, idx, src, axis=0):
    return tgt.at[idx].add(src)
def _segment_sum(src, seg, n):
    return jax.ops.segment_sum(src, seg, n)
class _Rng:
    def __init__(self, key):
        self._k = key
    def _next(self):
        self._k, sub = jax.random.split(self._k)
        return sub
    def normal(self, shape):
        return jax.random.normal(self._next(), shape, dtype=jnp.bfloat16)
    def randint(self, lo, hi, shape):
        return jax.random.randint(self._next(), shape, lo, hi, dtype=jnp.int32)
    def uniform(self, shape, lo=0.0, hi=1.0):
        return jax.random.uniform(self._next(), shape, jnp.bfloat16, lo, hi)
    def permutation(self, n):
        return jax.random.permutation(self._next(), n)


kernel_name = 'interleave_layers__sliding_local_dilated__linear_kernel_hedgehog__prompt'

def setup_inputs():
    _rng = _Rng(jax.random.key(int.from_bytes(__import__("os").urandom(4), "little")))
    _w = (lambda a: (lambda t: t.astype(jnp.bfloat16) if jnp.issubdtype(t.dtype, jnp.floating) else t)(jnp.asarray(a)))
    def _A_setup():
        B, S, D = 1, 2048, 1024
        return {
            "x": _w((lambda *s: _rng.normal(s) * 0.05)(B, S, D)),
            "wqkv": _w((lambda *s: _rng.normal(s) * 0.05)(D, 3 * D)),
            "wo": _w((lambda *s: _rng.normal(s) * 0.05)(D, D)),
        }
    _A_in = _A_setup()

    def _B_setup():
        B, S, D, H = 1, 2048, 1024, 32
        Dh = D // H
        return {
            "x": _w((lambda *s: _rng.normal(s) * 0.05)(B, S, D)),
            "wqkv": _w((lambda *s: _rng.normal(s) * 0.05)(D, 3 * D)),
            "w_phi": _w((lambda *s: _rng.normal(s) * 0.05)(H, Dh, Dh) * (Dh ** -0.5)),
            "wo": _w((lambda *s: _rng.normal(s) * 0.05)(D, D)),
        }
    _B_in = _B_setup()

    return {
        "A_x": _A_in["x"],
        "A_wqkv": _A_in["wqkv"],
        "A_wo": _A_in["wo"],
        "B_x": _B_in["x"],
        "B_wqkv": _B_in["wqkv"],
        "B_w_phi": _B_in["w_phi"],
        "B_wo": _B_in["wo"],
    }

def reference(A_x, A_wqkv, A_wo, B_x, B_wqkv, B_w_phi, B_wo):
    def _A_ref(x, wqkv, wo):
        B, S, D = x.shape
        H = 32; Dh = D // H
        W, dil = 8, 2
        qkv = (lambda x, *d: x.transpose(*d))((x @ wqkv).reshape(B, S, 3, H, Dh), 2, 0, 3, 1, 4)
        q, k, v = qkv[0], qkv[1], qkv[2]
        scale = Dh ** -0.5
        pos = jnp.arange(S)
        off = jnp.arange(W) * dil
        idx = pos[:, None] - off[None, :]
        mask = idx >= 0
        idx_c = jnp.where(mask, idx, 0).reshape(-1)
        kg = k[:, :, idx_c, :].reshape(B, H, S, W, Dh)
        vg = v[:, :, idx_c, :].reshape(B, H, S, W, Dh)
        logits = jnp.einsum("bhsd,bhswd->bhsw", q, kg) * scale
        logits = jnp.where(mask[None, None, :, :], logits, -1e9)
        attn = _softmax(logits, axis=-1)
        o = jnp.einsum("bhsw,bhswd->bhsd", attn, vg)
        return (lambda x, *d: x.transpose(*d))(o, 0, 2, 1, 3).reshape(B, S, D) @ wo

    def _B_ref(x, wqkv, w_phi, wo):
        B, S, D = x.shape
        H = 32; Dh = D // H
        qkv = (lambda x, *d: x.transpose(*d))((x @ wqkv).reshape(B, S, 3, H, Dh), 2, 0, 3, 1, 4)
        q, k, v = qkv[0], qkv[1], qkv[2]
        pq = jnp.einsum("bhsd,hdf->bhsf", q, w_phi)
        pk = jnp.einsum("bhsd,hdf->bhsf", k, w_phi)
        phi_q = jnp.concatenate([_softmax(pq, axis=-1), _softmax(-pq, axis=-1)], axis=-1)
        phi_k = jnp.concatenate([_softmax(pk, axis=-1), _softmax(-pk, axis=-1)], axis=-1)
        kv = jnp.einsum("bhsf,bhsd->bhfd", phi_k, v)
        z  = jnp.einsum("bhsf->bhf", phi_k)
        num = jnp.einsum("bhqf,bhfd->bhqd", phi_q, kv)
        den = jnp.einsum("bhqf,bhf->bhq", phi_q, z)[..., None] + 1e-6
        o = num / den
        return (lambda x, *d: x.transpose(*d))(o, 0, 2, 1, 3).reshape(B, S, D) @ wo

    x = A_x
    x = x + _A_ref(_layernorm(x, axis=-1), A_wqkv, A_wo)
    x = x + _B_ref(_layernorm(x, axis=-1), B_wqkv, B_w_phi, B_wo)
    x = x + _A_ref(_layernorm(x, axis=-1), A_wqkv, A_wo)
    x = x + _B_ref(_layernorm(x, axis=-1), B_wqkv, B_w_phi, B_wo)
    return x
```

```python
import jax
import jax.numpy as jnp
from jax import lax
import jax.experimental.pallas as pl
import jax.experimental.pallas.tpu as pltpu

S, D, H, DH = 2048, 1024, 32, 32
W, DIL = 8, 2
C = 256
NC = S // C
F32, BF16 = jnp.float32, jnp.bfloat16
NT = (((1,), (1,)), ((), ()))
RB = 64


def _mm(a, b):
    return jnp.dot(a, b, preferred_element_type=F32)


def _ln(x):
    m = jnp.mean(x, axis=0, keepdims=True)
    xc = x - m
    v = jnp.mean(xc * xc, axis=0, keepdims=True)
    return (xc * (1.0 / jnp.sqrt(v + 1e-5))).astype(BF16)


def _dual_softmax(p):
    pos, neg = [], []
    for h in range(4):
        ph = p[h * DH:(h + 1) * DH]
        ep = jnp.exp(ph - jnp.max(ph, axis=0, keepdims=True))
        en = jnp.exp(jnp.min(ph, axis=0, keepdims=True) - ph)
        pos.append(ep * (1.0 / jnp.sum(ep, axis=0, keepdims=True)))
        neg.append(en * (1.0 / jnp.sum(en, axis=0, keepdims=True)))
    return pos + neg


def _kernel(x_hbm, awqkv_hbm, awo_hbm, bwqkv_hbm, phi_hbm, bwo_hbm, o_hbm,
            xin, wqa, woa, wqb, wob, phi, xt, waT, woaT, wbT, wobT, tmp,
            kprev, vprev, ot, kvacc, zacc, kvT, obuf, sems, osem):
    cps = [pltpu.make_async_copy(s, d, sems.at[i]) for i, (s, d) in enumerate(
        [(x_hbm, xin), (awqkv_hbm, wqa), (awo_hbm, woa), (phi_hbm, phi),
         (bwqkv_hbm, wqb), (bwo_hbm, wob)])]
    for c in cps:
        c.start()

    cps[0].wait()

    def tx(c, _):
        r = pl.multiple_of(c * C, C)
        xt[c] = xin[pl.ds(r, C), :].astype(F32).T
    lax.fori_loop(0, NC, tx, None)

    cps[1].wait()
    for g in range(4):
        for p in range(3):
            col = p * D + g * 256
            for l in range(8):
                tmp[l * 256:(l + 1) * 256, :] = wqa[l * 128:(l + 1) * 128, col:col + 256].astype(F32).T
            for d in range(0, DH, 2):
                a = jnp.concatenate([tmp[pl.ds(l * 256 + d, 8, stride=DH), :] for l in range(8)], axis=1)
                b = jnp.concatenate([tmp[pl.ds(l * 256 + d + 1, 8, stride=DH), :] for l in range(8)], axis=1)
                waT[g, p * 256 + d * 8:p * 256 + d * 8 + 16, :] = (
                    jnp.concatenate([a, b], axis=0).astype(BF16))
    cps[2].wait()
    tmp2 = zacc
    for g in range(4):
        for l in range(8):
            tmp2[l] = woa[g * 256:(g + 1) * 256, l * 128:(l + 1) * 128].astype(F32)
            t = jnp.concatenate(
                [tmp2[l, pl.ds(d, 8, stride=DH), :] for d in range(DH)], axis=0)
            woaT[l * 128:(l + 1) * 128, g * 256:(g + 1) * 256] = t.T.astype(BF16)
    cps[3].wait()
    cps[4].wait()
    ri = lax.broadcasted_iota(jnp.int32, (128, 128), 0) // DH
    ci = lax.broadcasted_iota(jnp.int32, (128, 128), 1) // DH
    for g in range(8):
        ph = phi[g * 128:(g + 1) * 128, :].astype(F32)
        bd = jnp.where(ri == ci, jnp.concatenate([ph] * 4, axis=1), 0.0)
        bdT = bd.T.astype(BF16)
        for p in range(2):
            col = p * D + g * 128
            wbT[p, g * 128:(g + 1) * 128, :] = lax.dot_general(
                bdT, wqb[:, col:col + 128], NT, preferred_element_type=F32).astype(BF16)
        col = 2 * D + g * 128
        wbT[2, g * 128:(g + 1) * 128, :] = wqb[:, col:col + 128].astype(F32).T.astype(BF16)
    cps[5].wait()
    for g in range(8):
        wobT[g * 128:(g + 1) * 128, :] = wob[:, g * 128:(g + 1) * 128].astype(F32).T.astype(BF16)

    lane = lax.broadcasted_iota(jnp.int32, (8, 128), 1)
    laneb = lax.broadcasted_iota(jnp.int32, (RB, 128), 1)

    def shifted(cur, prev, w):
        if w == 0:
            return cur
        n = DIL * w
        u = pltpu.bitcast(cur, jnp.int32)
        up = pltpu.bitcast(prev, jnp.int32)
        m = laneb[:RB // 2] >= 128 - n
        return pltpu.bitcast(pltpu.roll(jnp.where(m, up, u), n, 1), BF16)

    def layer_a(c, x):
        ln = _ln(x)
        for g in range(4):
            qkv = _mm(waT[g], ln)
            q, k, v = (qkv[i * 256:(i + 1) * 256].astype(BF16) for i in range(3))
            rows = slice(g * 256, (g + 1) * 256)
            for j in range(C // 128):
                ls = slice(j * 128, (j + 1) * 128)
                lp = slice((j - 1) * 128, j * 128)
                acc = [None] * W
                for r in range(0, 256, RB):
                    rs = slice(r, r + RB)
                    kp = kprev[g * 256 + r:g * 256 + r + RB, :] if j == 0 else k[rs, lp]
                    qq = q[rs, ls].astype(F32)
                    kc = k[rs, ls]
                    for w in range(W):
                        pr = qq * shifted(kc, kp, w).astype(F32)
                        pr = jnp.sum(pr.reshape(RB // 8, 8, 128), axis=0)
                        acc[w] = pr if acc[w] is None else acc[w] + pr
                pos = c * C + j * 128 + lane
                lg = [acc[0] * DH ** -0.5] + [
                    jnp.where(pos >= DIL * w, acc[w] * DH ** -0.5, -1e9) for w in range(1, W)]
                mx = lg[0]
                for w in range(1, W):
                    mx = jnp.maximum(mx, lg[w])
                e = [jnp.exp(l - mx) for l in lg]
                inv = 1.0 / sum(e[1:], e[0])
                a = [(ei * inv)[None] for ei in e]
                for r in range(0, 256, RB):
                    rs = slice(r, r + RB)
                    vp = vprev[g * 256 + r:g * 256 + r + RB, :] if j == 0 else v[rs, lp]
                    vc = v[rs, ls]
                    o = None
                    for w in range(W):
                        t = a[w] * shifted(vc, vp, w).astype(F32).reshape(RB // 8, 8, 128)
                        o = t if o is None else o + t
                    ot[g * 256 + r:g * 256 + r + RB, ls] = o.reshape(RB, 128).astype(BF16)
            kprev[rows, :] = k[:, C - 128:]
            vprev[rows, :] = v[:, C - 128:]
        return x + _mm(woaT[...], ot[...])

    def layer_b1(x):
        ln = _ln(x)
        for g in range(4):
            rows = slice(g * 256, (g + 1) * 256)
            pk = _mm(wbT[1, rows, :], ln)
            v = _mm(wbT[2, rows, :], ln).astype(BF16)
            for s in range(2):
                f = jnp.concatenate(_dual_softmax(pk[s * 128:(s + 1) * 128]), axis=0)
                zs = f[:, :128]
                for j in range(1, C // 128):
                    zs = zs + f[:, j * 128:(j + 1) * 128]
                zacc[2 * g + s] += zs
                kvacc[2 * g + s] += lax.dot_general(
                    f.astype(BF16), v[s * 128:(s + 1) * 128], NT, preferred_element_type=F32)

    def finish_kv():
        r = lax.broadcasted_iota(jnp.int32, (144, 256), 0)
        cc = (lax.broadcasted_iota(jnp.int32, (144, 256), 1) % 128) // DH
        keep = jnp.where(r < 128, r // DH, r - 128) == cc
        for g in range(8):
            t = jnp.concatenate([kvacc[g].T, zacc[g].T[:16]], axis=0)
            z = jnp.sum(zacc[g].T, axis=0, keepdims=True)
            t = jnp.where(r < 128, t, z)
            kvT[g] = jnp.where(keep, t, 0.0)

    def layer_b2(x):
        ln = _ln(x)
        for g in range(4):
            rows = slice(g * 256, (g + 1) * 256)
            pq = _mm(wbT[0, rows, :], ln)
            for s in range(2):
                f = jnp.concatenate(_dual_softmax(pq[s * 128:(s + 1) * 128]), axis=0)
                nd = _mm(kvT[2 * g + s].astype(BF16), f.astype(BF16))
                inv = 1.0 / (nd[128:136] + 1e-6)
                for h in range(4):
                    r0 = g * 256 + s * 128 + h * DH
                    ot[r0:r0 + DH, :] = (nd[h * DH:(h + 1) * DH] * inv[h:h + 1]).astype(BF16)
        return x + _mm(wobT[...], ot[...])

    def reset():
        kprev[...] = jnp.zeros(kprev.shape, BF16)
        vprev[...] = jnp.zeros(vprev.shape, BF16)
        kvacc[...] = jnp.zeros(kvacc.shape, F32)
        zacc[...] = jnp.zeros(zacc.shape, F32)

    reset()

    def p1(c, _):
        xt[c] = layer_a(c, xt[c])
        layer_b1(xt[c])
    lax.fori_loop(0, NC, p1, None)
    finish_kv()
    reset()

    def p2(c, _):
        xt[c] = layer_a(c, layer_b2(xt[c]))
        layer_b1(xt[c])
    lax.fori_loop(0, NC, p2, None)
    finish_kv()

    def ocp(c):
        return pltpu.make_async_copy(
            obuf.at[c], o_hbm.at[pl.ds(pl.multiple_of(c * C, C), C), :], osem.at[c])

    def p3(c, _):
        obuf[c] = layer_b2(xt[c]).T.astype(BF16)
        ocp(c).start()
    lax.fori_loop(0, NC, p3, None)
    for c in range(NC):
        ocp(c).wait()


@jax.jit
def pallas_interleave_layers__sliding_local_dilated__linear_kernel_hedgehog__prompt_kernel(
    A_x, A_wqkv, A_wo, B_x, B_wqkv, B_w_phi, B_wo,
):
    hbm = pl.BlockSpec(memory_space=pl.ANY)
    vm = pltpu.VMEM
    out = pl.pallas_call(
        _kernel,
        in_specs=[hbm] * 6,
        out_specs=hbm,
        out_shape=jax.ShapeDtypeStruct((S, D), BF16),
        scratch_shapes=[
            vm((S, D), BF16), vm((D, 3 * D), BF16), vm((D, D), BF16),
            vm((D, 3 * D), BF16), vm((D, D), BF16), vm((D, DH), BF16),
            vm((NC, D, C), F32),
            vm((4, 768, D), BF16), vm((D, D), BF16), vm((3, D, D), BF16), vm((D, D), BF16),
            vm((2048, 128), F32),
            vm((D, 128), BF16), vm((D, 128), BF16), vm((D, C), BF16),
            vm((8, 256, 128), F32), vm((8, 256, 128), F32), vm((8, 144, 256), F32),
            vm((NC, C, D), BF16),
            pltpu.SemaphoreType.DMA((6,)), pltpu.SemaphoreType.DMA((NC,)),
        ],
        compiler_params=pltpu.CompilerParams(vmem_limit_bytes=110 * 1024 * 1024),
    )(A_x.reshape(S, D), A_wqkv, A_wo, B_wqkv, B_w_phi.reshape(H * DH, DH), B_wo)
    return out.reshape(1, S, D)
```

```python
import jax
import jax.numpy as jnp
from jax import lax
import jax.experimental.pallas as pl
import jax.experimental.pallas.tpu as pltpu

S, D, H, DH = 2048, 1024, 32, 32
W, DIL = 8, 2
C = 256
NC = S // C
F32, BF16 = jnp.float32, jnp.bfloat16
NT = (((1,), (1,)), ((), ()))
RB = 64


def _mm(a, b):
    return jnp.dot(a, b, preferred_element_type=F32)


def _ln(x):
    m = jnp.mean(x, axis=0, keepdims=True)
    xc = x - m
    v = jnp.mean(xc * xc, axis=0, keepdims=True)
    return (xc * (1.0 / jnp.sqrt(v + 1e-5))).astype(BF16)


def _dual_softmax(p):
    pos, neg = [], []
    for h in range(4):
        ph = p[h * DH:(h + 1) * DH]
        ep = jnp.exp(ph - jnp.max(ph, axis=0, keepdims=True))
        en = jnp.exp(jnp.min(ph, axis=0, keepdims=True) - ph)
        pos.append(ep * (1.0 / jnp.sum(ep, axis=0, keepdims=True)))
        neg.append(en * (1.0 / jnp.sum(en, axis=0, keepdims=True)))
    return pos + neg


def _kernel(x_hbm, awqkv_hbm, awo_hbm, bwqkv_hbm, phi_hbm, bwo_hbm, o_hbm,
            xin, wqa, woa, wqb, wob, phi, xt, lnt, waT, woaT, wbT, wobT, tmp, qb,
            kprev, vprev, ot, kvacc, zacc, kvT, obuf, xsem, asem, sems, osem):
    def ds(i, n):
        return pl.ds(i * n if isinstance(i, int) else pl.multiple_of(i * n, n), n)

    def xcp(c):
        return pltpu.make_async_copy(x_hbm.at[ds(c, 512), :], xin.at[ds(c, 512), :], xsem.at[c])

    def acp(g, p):
        cols = ds(4 * p + g, 256)
        return pltpu.make_async_copy(awqkv_hbm.at[:, cols], wqa.at[:, cols], asem.at[g, p])

    cps = [pltpu.make_async_copy(s, d, sems.at[i]) for i, (s, d) in enumerate(
        [(awo_hbm, woa), (phi_hbm, phi), (bwqkv_hbm, wqb), (bwo_hbm, wob)])]
    xcp(0).start()
    for p in range(3):
        acp(0, p).start()
    xcp(1).start()

    def prep_a(g, l, u):
        for p in range(3):
            t0 = (3 * u + p)
            tmp[t0] = wqa[ds(l, 128), ds(4 * p + g, 256)].astype(F32).T
            t = jnp.concatenate([tmp[t0, pl.ds(d, 8, stride=DH), :] for d in range(DH)], axis=0)
            waT[g, p * 256:(p + 1) * 256, ds(l, 128)] = t.astype(BF16)

    def prep_woa(l, u):
        for g in range(4):
            t0 = (4 * u + g)
            tmp[t0] = woa[g * 256:(g + 1) * 256, ds(l, 128)].astype(F32)
            t = jnp.concatenate([tmp[t0, pl.ds(d, 8, stride=DH), :] for d in range(DH)], axis=0)
            woaT[g, ds(l, 128), :] = t.T.astype(BF16)

    def prep_phi(g, p):
        ri = lax.broadcasted_iota(jnp.int32, (128, 128), 0) // DH
        ci = lax.broadcasted_iota(jnp.int32, (128, 128), 1) // DH
        ph = phi[ds(g, 128), :].astype(F32)
        bd = jnp.where(ri == ci, jnp.concatenate([ph] * 4, axis=1), 0.0)
        wbT[p, ds(g, 128), :] = lax.dot_general(
            bd.T.astype(BF16), wqb[:, ds(8 * p + g, 128)], NT,
            preferred_element_type=F32).astype(BF16)

    lane = lax.broadcasted_iota(jnp.int32, (8, 128), 1)
    laneb = lax.broadcasted_iota(jnp.int32, (RB, 128), 1)

    def shifted(cur, prev, w):
        if w == 0:
            return cur
        n = DIL * w
        u = pltpu.bitcast(cur, jnp.int32)
        up = pltpu.bitcast(prev, jnp.int32)
        m = laneb[:RB // 2] >= 128 - n
        return pltpu.bitcast(pltpu.roll(jnp.where(m, up, u), n, 1), BF16)

    def proj(g, ln):
        return _mm(waT[g], ln).astype(BF16)

    def attn(c, q, k, v, out, kprev, vprev):
        if True:
            for j in range(C // 128):
                ls = slice(j * 128, (j + 1) * 128)
                lp = slice((j - 1) * 128, j * 128)
                acc = [None] * W
                for r in range(0, 256, RB):
                    rs = slice(r, r + RB)
                    kp = kprev[rs, :] if j == 0 else k[rs, lp]
                    qq = q[rs, ls].astype(F32)
                    kc = k[rs, ls]
                    for w in range(W):
                        pr = qq * shifted(kc, kp, w).astype(F32)
                        pr = jnp.sum(pr.reshape(RB // 8, 8, 128), axis=0)
                        acc[w] = pr if acc[w] is None else acc[w] + pr
                pos = c * C + j * 128 + lane
                lg = [acc[0] * DH ** -0.5] + [
                    jnp.where(pos >= DIL * w, acc[w] * DH ** -0.5, -1e9) for w in range(1, W)]
                mx = lg[0]
                for w in range(1, W):
                    mx = jnp.maximum(mx, lg[w])
                e = [jnp.exp(l - mx) for l in lg]
                inv = 1.0 / sum(e[1:], e[0])
                a = [(ei * inv)[None] for ei in e]
                for r in range(0, 256, RB):
                    rs = slice(r, r + RB)
                    vp = vprev[rs, :] if j == 0 else v[rs, lp]
                    vc = v[rs, ls]
                    o = None
                    for w in range(W):
                        t = a[w] * shifted(vc, vp, w).astype(F32).reshape(RB // 8, 8, 128)
                        o = t if o is None else o + t
                    out(r, ls, o.reshape(RB, 128).astype(BF16))
            kprev[...] = k[:, C - 128:]
            vprev[...] = v[:, C - 128:]

    def attn_all(c, u):
        ln = _ln(xt[c])
        for g in range(4):
            def out(r, ls, val):
                ot[u, g * 256 + r:g * 256 + r + RB, ls] = val
            qkv = proj(g, ln)
            attn(c, qkv[:256], qkv[256:512], qkv[512:], out, kprev.at[g], vprev.at[g])

    def out_a(c, u):
        w = jnp.concatenate([woaT[g] for g in range(4)], axis=1)
        x = xt[c] + _mm(w, ot[u])
        xt[c] = x
        lnt[c] = _ln(x)

    def layer_b1(c):
        ln = lnt[c]
        for g in range(4):
            rows = slice(g * 256, (g + 1) * 256)
            pk = _mm(wbT[1, rows, :], ln)
            v = _mm(wbT[2, rows, :], ln).astype(BF16)
            for s in range(2):
                f = jnp.concatenate(_dual_softmax(pk[s * 128:(s + 1) * 128]), axis=0)
                zs = f[:, :128]
                for j in range(1, C // 128):
                    zs = zs + f[:, j * 128:(j + 1) * 128]
                zacc[2 * g + s] += zs
                kvacc[2 * g + s] += lax.dot_general(
                    f.astype(BF16), v[s * 128:(s + 1) * 128], NT, preferred_element_type=F32)

    def finish_kv():
        r = lax.broadcasted_iota(jnp.int32, (144, 256), 0)
        cc = (lax.broadcasted_iota(jnp.int32, (144, 256), 1) % 128) // DH
        keep = jnp.where(r < 128, r // DH, r - 128) == cc
        for g in range(8):
            t = jnp.concatenate([kvacc[g].T, zacc[g].T[:16]], axis=0)
            z = jnp.sum(zacc[g].T, axis=0, keepdims=True)
            t = jnp.where(r < 128, t, z)
            kvT[g] = jnp.where(keep, t, 0.0)

    def layer_b2(c, u):
        ln = lnt[c]
        for g in range(4):
            rows = slice(g * 256, (g + 1) * 256)
            pq = _mm(wbT[0, rows, :], ln)
            for s in range(2):
                f = jnp.concatenate(_dual_softmax(pq[s * 128:(s + 1) * 128]), axis=0)
                nd = _mm(kvT[2 * g + s].astype(BF16), f.astype(BF16))
                inv = 1.0 / (nd[128:136] + 1e-6)
                for h in range(4):
                    r0 = g * 256 + s * 128 + h * DH
                    ot[u, r0:r0 + DH, :] = (nd[h * DH:(h + 1) * DH] * inv[h:h + 1]).astype(BF16)
        return xt[c] + _mm(wobT[...], ot[u])

    def reset():
        kprev[...] = jnp.zeros(kprev.shape, BF16)
        vprev[...] = jnp.zeros(vprev.shape, BF16)
        kvacc[...] = jnp.zeros(kvacc.shape, F32)
        zacc[...] = jnp.zeros(zacc.shape, F32)

    reset()
    for p in range(3):
        acp(0, p).wait()
    for l in range(8):
        prep_a(0, l, l % 2)

    def tx(c):
        pass
        for r in range(0, D, 256):
            xt[c, r:r + 256, :] = xin[ds(c, C), r:r + 256].astype(F32).T
        lnt[c] = _ln(xt[c])

    xcp(0).wait()
    for c in range(2, 4):
        xcp(c).start()
    for p in range(3):
        acp(1, p).start()
    tx(0)

    tx(1)
    qb[0] = proj(0, lnt[0])

    def step(t, u, mode):
        g, c = t // NC, t % NC

        def out(r, ls, val):
            ot[c, ds(4 * g + r // RB, RB), ls] = val
        qb[1 - u] = proj(jnp.minimum(t + 1, 4 * NC - 1) // NC, lnt[(t + 1) % NC])
        attn(c, qb[u, 0:0 + 256, :], qb[u, 256:256 + 256, :], qb[u, 512:512 + 256, :],
             out, kprev.at[0], vprev.at[0])
        if mode == 2:
            prep_woa(c, u)

    def g0(i, _):
        @pl.when(i < 3)
        def _():
            xcp(i + 1).wait()
        for u in range(2):
            step(2 * i + u, u, 0)
            tx(jnp.minimum(2 * i + u + 2, NC - 1))
    lax.fori_loop(0, 4, g0, None)
    for p in range(3):
        acp(1, p).wait()
    for g in range(2, 4):
        for p in range(3):
            acp(g, p).start()

    def pa(l, _):
        prep_a(1, l, 0)
    lax.fori_loop(0, 8, pa, None)
    qb[0] = proj(1, lnt[0])
    for cp in cps:
        cp.start()

    def g1(i, _):
        @pl.when(i % 4 == 0)
        def _():
            for p in range(3):
                acp(i // 4 + 1, p).wait()
        for u in range(2):
            t = 2 * i + u
            prep_a(jnp.minimum(t // NC + 1, 3), t % NC, u)
            step(t, u, 1)
    lax.fori_loop(4, 12, g1, None)

    for cp in cps:
        cp.wait()

    def g3(i, _):
        for u in range(2):
            step(2 * i + u, u, 2)
    lax.fori_loop(12, 16, g3, None)

    reset()

    def p0(i, _):
        for u in range(4):
            c = 4 * i + u
            out_a(c, c)
            prep_phi(c, 1)
            wbT[2, ds(c, 128), :] = wqb[:, ds(16 + c, 128)].astype(F32).T.astype(BF16)
    lax.fori_loop(0, NC // 4, p0, None)

    def p1(i, _):
        for u in range(2):
            c = 2 * i + u
            layer_b1(c)
            prep_phi(c, 0)
            wobT[ds(c, 128), :] = wob[:, ds(c, 128)].astype(F32).T.astype(BF16)
    lax.fori_loop(0, NC // 2, p1, None)
    finish_kv()
    reset()

    def p2(i, _):
        for u in range(2):
            xt[2 * i + u] = layer_b2(2 * i + u, u)
        for u in range(2):
            attn_all(2 * i + u, u)
        for u in range(2):
            out_a(2 * i + u, u)
        for u in range(2):
            layer_b1(2 * i + u)
    lax.fori_loop(0, NC // 2, p2, None)
    finish_kv()

    def ocp(c):
        return pltpu.make_async_copy(obuf.at[c], o_hbm.at[ds(c, C), :], osem.at[c])

    def p3(i, _):
        for u in range(2):
            obuf[2 * i + u] = layer_b2(2 * i + u, u).T.astype(BF16)
        for u in range(2):
            ocp(2 * i + u).start()
    lax.fori_loop(0, NC // 2, p3, None)
    for c in range(NC):
        ocp(c).wait()


@jax.jit
def pallas_interleave_layers__sliding_local_dilated__linear_kernel_hedgehog__prompt_kernel(
    A_x, A_wqkv, A_wo, B_x, B_wqkv, B_w_phi, B_wo,
):
    hbm = pl.BlockSpec(memory_space=pl.ANY)
    vm = pltpu.VMEM
    out = pl.pallas_call(
        _kernel,
        in_specs=[hbm] * 6,
        out_specs=hbm,
        out_shape=jax.ShapeDtypeStruct((S, D), BF16),
        scratch_shapes=[
            vm((S, D), BF16), vm((D, 3 * D), BF16), vm((D, D), BF16),
            vm((D, 3 * D), BF16), vm((D, D), BF16), vm((D, DH), BF16),
            vm((NC, D, C), F32), vm((NC, D, C), BF16),
            vm((4, 768, D), BF16), vm((4, D, 256), BF16), vm((3, D, D), BF16), vm((D, D), BF16),
            vm((8, 256, 128), F32), vm((2, 768, C), BF16),
            vm((4, 256, 128), BF16), vm((4, 256, 128), BF16), vm((NC, D, C), BF16),
            vm((8, 256, 128), F32), vm((8, 256, 128), F32), vm((8, 144, 256), F32),
            vm((NC, C, D), BF16),
            pltpu.SemaphoreType.DMA((4,)), pltpu.SemaphoreType.DMA((4, 3)),
            pltpu.SemaphoreType.DMA((4,)), pltpu.SemaphoreType.DMA((NC,)),
        ],
        compiler_params=pltpu.CompilerParams(vmem_limit_bytes=110 * 1024 * 1024),
    )(A_x.reshape(S, D), A_wqkv, A_wo, B_wqkv, B_w_phi.reshape(H * DH, DH), B_wo)
    return out.reshape(1, S, D)
```

```python
import jax
import jax.numpy as jnp
from jax import lax
import jax.experimental.pallas as pl
import jax.experimental.pallas.tpu as pltpu

S, D, H, DH = 2048, 1024, 32, 32
W, DIL = 8, 2
C = 256
NC = S // C
F32, BF16 = jnp.float32, jnp.bfloat16
NT = (((1,), (1,)), ((), ()))
RB = 64


def _mm(a, b):
    return jnp.dot(a, b, preferred_element_type=F32)


def _rcp(s):
    r = pl.reciprocal(s, approx=True)
    return r * (2.0 - s * r)


def _ln(x):
    m = jnp.mean(x, axis=0, keepdims=True)
    xc = x - m
    v = jnp.mean(xc * xc, axis=0, keepdims=True)
    return (xc * (1.0 / jnp.sqrt(v + 1e-5))).astype(BF16)


def _dual_softmax(p):
    pos, neg = [], []
    p = p * 1.4426950408889634
    for h in range(4):
        ph = p[h * DH:(h + 1) * DH]
        ep = jnp.exp2(ph - jnp.max(ph, axis=0, keepdims=True))
        en = jnp.exp2(jnp.min(ph, axis=0, keepdims=True) - ph)
        pos.append(ep * (_rcp(jnp.sum(ep, axis=0, keepdims=True))))
        neg.append(en * (_rcp(jnp.sum(en, axis=0, keepdims=True))))
    return pos + neg


def _kernel(x_hbm, awqkv_hbm, awo_hbm, bwqkv_hbm, phi_hbm, bwo_hbm, o_hbm,
            xin, wqa, woa, wqb, wob, phi, xt, lnt, waT, woaT, wbT, wobT, tmp, qb,
            kprev, vprev, ot, kvacc, zacc, kvT, obuf, xsem, asem, sems, osem):
    def ds(i, n):
        return pl.ds(i * n if isinstance(i, int) else pl.multiple_of(i * n, n), n)

    def xcp(c):
        return pltpu.make_async_copy(x_hbm.at[ds(c, 512), :], xin.at[ds(c, 512), :], xsem.at[c])

    def acp(g, p):
        cols = ds(4 * p + g, 256)
        return pltpu.make_async_copy(awqkv_hbm.at[:, cols], wqa.at[:, cols], asem.at[g, p])

    cps = [pltpu.make_async_copy(s, d, sems.at[i]) for i, (s, d) in enumerate(
        [(awo_hbm, woa), (phi_hbm, phi), (bwqkv_hbm, wqb), (bwo_hbm, wob)])]
    xcp(0).start()
    for p in range(3):
        acp(0, p).start()
    xcp(1).start()

    def prep_a(g, l, u):
        for p in range(3):
            t0 = (3 * u + p)
            tmp[t0] = wqa[ds(l, 128), ds(4 * p + g, 256)].astype(F32).T
            t = jnp.concatenate([tmp[t0, pl.ds(d, 8, stride=DH), :] for d in range(DH)], axis=0)
            waT[g, p * 256:(p + 1) * 256, ds(l, 128)] = t.astype(BF16)

    def prep_woa(l, u):
        for g in range(4):
            t0 = (4 * u + g)
            tmp[t0] = woa[g * 256:(g + 1) * 256, ds(l, 128)].astype(F32)
            t = jnp.concatenate([tmp[t0, pl.ds(d, 8, stride=DH), :] for d in range(DH)], axis=0)
            woaT[g, ds(l, 128), :] = t.T.astype(BF16)

    def prep_phi(g, p):
        ri = lax.broadcasted_iota(jnp.int32, (128, 128), 0) // DH
        ci = lax.broadcasted_iota(jnp.int32, (128, 128), 1) // DH
        ph = phi[ds(g, 128), :].astype(F32)
        bd = jnp.where(ri == ci, jnp.concatenate([ph] * 4, axis=1), 0.0)
        wbT[p, ds(g, 128), :] = lax.dot_general(
            bd.T.astype(BF16), wqb[:, ds(8 * p + g, 128)], NT,
            preferred_element_type=F32).astype(BF16)

    lane = lax.broadcasted_iota(jnp.int32, (8, 128), 1)
    laneb = lax.broadcasted_iota(jnp.int32, (RB, 128), 1)

    def shifted(cur, prev, w):
        if w == 0:
            return cur
        n = DIL * w
        u = pltpu.bitcast(cur, jnp.int32)
        up = pltpu.bitcast(prev, jnp.int32)
        m = laneb[:RB // 2] >= 128 - n
        return pltpu.bitcast(pltpu.roll(jnp.where(m, up, u), n, 1), BF16)

    def proj(g, ln):
        return _mm(waT[g], ln).astype(BF16)

    def attn(c, q, k, v, out, kprev, vprev):
        if True:
            for j in range(C // 128):
                ls = slice(j * 128, (j + 1) * 128)
                lp = slice((j - 1) * 128, j * 128)
                acc = [None] * W
                for r in range(0, 256, RB):
                    rs = slice(r, r + RB)
                    kp = kprev[rs, :] if j == 0 else k[rs, lp]
                    qq = q[rs, ls].astype(F32)
                    kc = k[rs, ls]
                    for w in range(W):
                        pr = qq * shifted(kc, kp, w).astype(F32)
                        pr = jnp.sum(pr.reshape(RB // 8, 8, 128), axis=0)
                        acc[w] = pr if acc[w] is None else acc[w] + pr
                pos = c * C + j * 128 + lane
                lg = [acc[0] * DH ** -0.5] + [
                    jnp.where(pos >= DIL * w, acc[w] * DH ** -0.5, -1e9) for w in range(1, W)]
                mx = lg[0]
                for w in range(1, W):
                    mx = jnp.maximum(mx, lg[w])
                e = [jnp.exp(l - mx) for l in lg]
                inv = _rcp(sum(e[1:], e[0]))
                a = [(ei * inv)[None] for ei in e]
                for r in range(0, 256, RB):
                    rs = slice(r, r + RB)
                    vp = vprev[rs, :] if j == 0 else v[rs, lp]
                    vc = v[rs, ls]
                    o = None
                    for w in range(W):
                        t = a[w] * shifted(vc, vp, w).astype(F32).reshape(RB // 8, 8, 128)
                        o = t if o is None else o + t
                    out(r, ls, o.reshape(RB, 128).astype(BF16))
            kprev[...] = k[:, C - 128:]
            vprev[...] = v[:, C - 128:]

    def out_a(c, u):
        w = jnp.concatenate([woaT[g] for g in range(4)], axis=1)
        x = xt[c] + _mm(w, ot[u])
        xt[c] = x
        lnt[c] = _ln(x)

    def layer_b1(c):
        ln = lnt[c]
        pks = [_mm(wbT[1, g * 256:(g + 1) * 256, :], ln) for g in range(4)]
        for g in range(4):
            rows = slice(g * 256, (g + 1) * 256)
            pk = pks[g]
            v = _mm(wbT[2, rows, :], ln).astype(BF16)
            for s in range(2):
                f = jnp.concatenate(_dual_softmax(pk[s * 128:(s + 1) * 128]), axis=0)
                zs = f[:, :128]
                for j in range(1, C // 128):
                    zs = zs + f[:, j * 128:(j + 1) * 128]
                zacc[2 * g + s] += zs
                kvacc[2 * g + s] += lax.dot_general(
                    f.astype(BF16), v[s * 128:(s + 1) * 128], NT, preferred_element_type=F32)

    def finish_kv():
        r = lax.broadcasted_iota(jnp.int32, (144, 256), 0)
        cc = (lax.broadcasted_iota(jnp.int32, (144, 256), 1) % 128) // DH
        keep = jnp.where(r < 128, r // DH, r - 128) == cc
        for g in range(8):
            t = jnp.concatenate([kvacc[g].T, zacc[g].T[:16]], axis=0)
            z = jnp.sum(zacc[g].T, axis=0, keepdims=True)
            t = jnp.where(r < 128, t, z)
            kvT[g] = jnp.where(keep, t, 0.0)

    def layer_b2(c, u):
        ln = lnt[c]
        pqs = [_mm(wbT[0, g * 256:(g + 1) * 256, :], ln) for g in range(4)]
        for g in range(4):
            rows = slice(g * 256, (g + 1) * 256)
            pq = pqs[g]
            for s in range(2):
                f = jnp.concatenate(_dual_softmax(pq[s * 128:(s + 1) * 128]), axis=0)
                nd = _mm(kvT[2 * g + s].astype(BF16), f.astype(BF16))
                inv = 1.0 / (nd[128:136] + 1e-6)
                for h in range(4):
                    r0 = g * 256 + s * 128 + h * DH
                    ot[u, r0:r0 + DH, :] = (nd[h * DH:(h + 1) * DH] * inv[h:h + 1]).astype(BF16)
        return xt[c] + _mm(wobT[...], ot[u])

    def reset():
        kprev[...] = jnp.zeros(kprev.shape, BF16)
        vprev[...] = jnp.zeros(vprev.shape, BF16)
        kvacc[...] = jnp.zeros(kvacc.shape, F32)
        zacc[...] = jnp.zeros(zacc.shape, F32)

    reset()
    for p in range(3):
        acp(0, p).wait()

    def pb(l, _):
        prep_a(0, l, 0)
        prep_a(0, l + 4, 1)
    lax.fori_loop(0, 4, pb, None)

    def tx(c):
        pass
        for r in range(0, D, 256):
            xt[c, r:r + 256, :] = xin[ds(c, C), r:r + 256].astype(F32).T
        lnt[c] = _ln(xt[c])

    xcp(0).wait()
    for c in range(2, 4):
        xcp(c).start()
    for p in range(3):
        acp(1, p).start()
    tx(0)

    tx(1)
    qb[0] = proj(0, lnt[0])

    def step(t, u, mode):
        g, c = t // NC, t % NC

        def out(r, ls, val):
            ot[c, ds(4 * g + r // RB, RB), ls] = val
        qb[1 - u] = proj(jnp.minimum(t + 1, 4 * NC - 1) // NC, lnt[(t + 1) % NC])
        attn(c, qb[u, 0:0 + 256, :], qb[u, 256:256 + 256, :], qb[u, 512:512 + 256, :],
             out, kprev.at[0], vprev.at[0])
        if mode == 2:
            prep_woa(c, u)

    def g0(i, _):
        @pl.when(i < 3)
        def _():
            xcp(i + 1).wait()

        @pl.when(i == 3)
        def _():
            for p in range(3):
                acp(1, p).wait()
            for g in range(2, 4):
                for p in range(3):
                    acp(g, p).start()

            def pa(l, _):
                prep_a(1, l, 0)
                prep_a(1, l + 4, 1)
            with jax.named_scope('ph_pa'):
                lax.fori_loop(0, 4, pa, None)
        for u in range(2):
            step(2 * i + u, u, 0)
            tx(jnp.minimum(2 * i + u + 2, NC - 1))
    with jax.named_scope('ph_g0'):
        lax.fori_loop(0, 4, g0, None)
    for cp in cps:
        cp.start()

    def g1(i, _):
        @pl.when(i % 4 == 0)
        def _():
            for p in range(3):
                acp(i // 4 + 1, p).wait()
        for u in range(2):
            t = 2 * i + u
            prep_a(jnp.minimum(t // NC + 1, 3), t % NC, u)
            step(t, u, 1)
    with jax.named_scope('ph_g1'):
        lax.fori_loop(4, 12, g1, None)

    for cp in cps:
        cp.wait()

    def g3(i, _):
        for u in range(2):
            step(2 * i + u, u, 2)
    with jax.named_scope('ph_g3'):
        lax.fori_loop(12, 16, g3, None)

    reset()

    def p0(i, _):
        for u in range(4):
            c = 4 * i + u
            out_a(c, c)
            prep_phi(c, 1)
            wbT[2, ds(c, 128), :] = wqb[:, ds(16 + c, 128)].astype(F32).T.astype(BF16)
    with jax.named_scope('ph_p0'):
        lax.fori_loop(0, NC // 4, p0, None)

    def p1(i, _):
        for u in range(2):
            c = 2 * i + u
            layer_b1(c)
            prep_phi(c, 0)
            wobT[ds(c, 128), :] = wob[:, ds(c, 128)].astype(F32).T.astype(BF16)
    with jax.named_scope('ph_p1'):
        lax.fori_loop(0, NC // 2, p1, None)
    finish_kv()
    reset()

    def p2(i, _):
        for u in range(2):
            c = 2 * i + u
            x = layer_b2(c, u)
            xt[c] = x
            lnt[c] = _ln(x)
    with jax.named_scope('ph_p2'):
        lax.fori_loop(0, NC // 2, p2, None)
    qb[0] = proj(0, lnt[0])

    def g4(i, _):
        for u in range(2):
            step(2 * i + u, u, 1)
    with jax.named_scope('ph_g4'):
        lax.fori_loop(0, 16, g4, None)

    def p4(i, _):
        for u in range(4):
            out_a(4 * i + u, 4 * i + u)
    with jax.named_scope('ph_p4'):
        lax.fori_loop(0, NC // 4, p4, None)

    def p5(i, _):
        for u in range(2):
            layer_b1(2 * i + u)
    with jax.named_scope('ph_p5'):
        lax.fori_loop(0, NC // 2, p5, None)
    finish_kv()

    def ocp(c):
        return pltpu.make_async_copy(obuf.at[c], o_hbm.at[ds(c, C), :], osem.at[c])

    def p3(i, _):
        for u in range(2):
            obuf[2 * i + u] = layer_b2(2 * i + u, u).T.astype(BF16)
        for u in range(2):
            ocp(2 * i + u).start()
    with jax.named_scope('ph_p3'):
        lax.fori_loop(0, NC // 2, p3, None)
    for c in range(NC):
        ocp(c).wait()


@jax.jit
def pallas_interleave_layers__sliding_local_dilated__linear_kernel_hedgehog__prompt_kernel(
    A_x, A_wqkv, A_wo, B_x, B_wqkv, B_w_phi, B_wo,
):
    hbm = pl.BlockSpec(memory_space=pl.ANY)
    vm = pltpu.VMEM
    out = pl.pallas_call(
        _kernel,
        in_specs=[hbm] * 6,
        out_specs=hbm,
        out_shape=jax.ShapeDtypeStruct((S, D), BF16),
        scratch_shapes=[
            vm((S, D), BF16), vm((D, 3 * D), BF16), vm((D, D), BF16),
            vm((D, 3 * D), BF16), vm((D, D), BF16), vm((D, DH), BF16),
            vm((NC, D, C), F32), vm((NC, D, C), BF16),
            vm((4, 768, D), BF16), vm((4, D, 256), BF16), vm((3, D, D), BF16), vm((D, D), BF16),
            vm((8, 256, 128), F32), vm((2, 768, C), BF16),
            vm((4, 256, 128), BF16), vm((4, 256, 128), BF16), vm((NC, D, C), BF16),
            vm((8, 256, 128), F32), vm((8, 256, 128), F32), vm((8, 144, 256), F32),
            vm((NC, C, D), BF16),
            pltpu.SemaphoreType.DMA((4,)), pltpu.SemaphoreType.DMA((4, 3)),
            pltpu.SemaphoreType.DMA((4,)), pltpu.SemaphoreType.DMA((NC,)),
        ],
        compiler_params=pltpu.CompilerParams(vmem_limit_bytes=110 * 1024 * 1024),
    )(A_x.reshape(S, D), A_wqkv, A_wo, B_wqkv, B_w_phi.reshape(H * DH, DH), B_wo)
    return out.reshape(1, S, D)
```
